```python
import os as _os
_os.environ.setdefault("JAX_PLATFORMS", "cpu")
import jax
import jax.numpy as jnp

def _softmax(x, axis=-1):
    return jax.nn.softmax(x, axis=axis)
def _gelu(x):
    return jax.nn.gelu(x, approximate=True)
def _silu(x):
    return jax.nn.silu(x)
def _sigmoid(x):
    return jax.nn.sigmoid(x)
def _layernorm(x, axis=-1, eps=1e-5):
    m = jnp.mean(x, axis=axis, keepdims=True)
    v = jnp.var(x, axis=axis, keepdims=True)
    return (x - m) / jnp.sqrt(v + eps)
def _scatter_add(tgt, idx, src, axis=0):
    return tgt.at[idx].add(src)
def _segment_sum(src, seg, n):
    return jax.ops.segment_sum(src, seg, n)
class _Rng:
    def __init__(self, key):
        self._k = key
    def _next(self):
        self._k, sub = jax.random.split(self._k)
        return sub
    def normal(self, shape):
        return jax.random.normal(self._next(), shape, dtype=jnp.bfloat16)
    def randint(self, lo, hi, shape):
        return jax.random.randint(self._next(), shape, lo, hi, dtype=jnp.int32)
    def uniform(self, shape, lo=0.0, hi=1.0):
        return jax.random.uniform(self._next(), shape, jnp.bfloat16, lo, hi)
    def permutation(self, n):
        return jax.random.permutation(self._next(), n)


kernel_name = 'concat_heads__mha_block_cached__gqa_block_cached__near_ridge'

def setup_inputs():
    _rng = _Rng(jax.random.key(int.from_bytes(__import__("os").urandom(4), "little")))
    _w = (lambda a: (lambda t: t.astype(jnp.bfloat16) if jnp.issubdtype(t.dtype, jnp.floating) else t)(jnp.asarray(a)))
    def _A_setup():
        B, Sq, D = 8, 128, 512
        H, Sk, Dh = 32, 1024, 128
        return {
            "x": _w((lambda *s: _rng.normal(s) * 0.8)(B, Sq, D)),
            "k_cache": _w((lambda *s: _rng.normal(s) * 0.8)(B, H, Sk, Dh)),
            "v_cache": _w((lambda *s: _rng.normal(s) * 0.05)(B, H, Sk, Dh)),
            "wq": _w((lambda *s: _rng.normal(s) * 0.8)(D, H * Dh) * (D ** -0.5)),
            "wo": _w((lambda *s: _rng.normal(s) * 0.05)(H * Dh, D) * ((H * Dh) ** -0.5)),
        }
    _A_in = _A_setup()

    def _B_setup():
        B, Sq, D = 8, 128, 512
        Hq, Hkv, Sk, Dh = 32, 32, 1024, 128
        assert Hq % Hkv == 0, (Hq, Hkv)
        return {
            "x": _w((lambda *s: _rng.normal(s) * 0.8)(B, Sq, D)),
            "k_cache": _w((lambda *s: _rng.normal(s) * 0.8)(B, Hkv, Sk, Dh)),
            "v_cache": _w((lambda *s: _rng.normal(s) * 0.05)(B, Hkv, Sk, Dh)),
            "wq": _w((lambda *s: _rng.normal(s) * 0.8)(D, Hq * Dh) * (D ** -0.5)),
            "wo": _w((lambda *s: _rng.normal(s) * 0.05)(Hq * Dh, D) * ((Hq * Dh) ** -0.5)),
        }
    _B_in = _B_setup()

    return {
        "A_x": _A_in["x"],
        "A_k_cache": _A_in["k_cache"],
        "A_v_cache": _A_in["v_cache"],
        "A_wq": _A_in["wq"],
        "A_wo": _A_in["wo"],
        "B_x": _B_in["x"],
        "B_k_cache": _B_in["k_cache"],
        "B_v_cache": _B_in["v_cache"],
        "B_wq": _B_in["wq"],
        "B_wo": _B_in["wo"],
    }

def reference(A_x, A_k_cache, A_v_cache, A_wq, A_wo, B_x, B_k_cache, B_v_cache, B_wq, B_wo):
    def _A_ref(x, k_cache, v_cache, wq, wo):
        B, Sq, D = x.shape
        H, Dh = 32, 128
        q = (lambda x, *d: x.transpose(*d))((x @ wq).reshape(B, Sq, H, Dh), 0, 2, 1, 3)
        scores = jnp.einsum("bhqd,bhkd->bhqk", q, k_cache) * (Dh ** -0.5)
        p = _softmax(scores, axis=-1)
        o = jnp.einsum("bhqk,bhkd->bhqd", p, v_cache)
        return (lambda x, *d: x.transpose(*d))(o, 0, 2, 1, 3).reshape(B, Sq, H * Dh) @ wo

    def _B_ref(x, k_cache, v_cache, wq, wo):
        B, Sq, D = x.shape
        Hq, Dh = 32, 128
        Hkv = k_cache.shape[1]
        rep = Hq // Hkv
        q = (lambda x, *d: x.transpose(*d))((x @ wq).reshape(B, Sq, Hq, Dh), 0, 2, 1, 3)
        k = jnp.repeat(k_cache, rep, axis=1)
        v = jnp.repeat(v_cache, rep, axis=1)
        scores = jnp.einsum("bhqd,bhkd->bhqk", q, k) * (Dh ** -0.5)
        p = _softmax(scores, axis=-1)
        o = jnp.einsum("bhqk,bhkd->bhqd", p, v)
        return (lambda x, *d: x.transpose(*d))(o, 0, 2, 1, 3).reshape(B, Sq, Hq * Dh) @ wo

    a = _A_ref(A_x, A_k_cache, A_v_cache, A_wq, A_wo)
    b = _B_ref(B_x, B_k_cache, B_v_cache, B_wq, B_wo)
    return jnp.concatenate([a, b], axis=-1)
```

```python
import math

import jax
import jax.numpy as jnp
import jax.experimental.pallas as pl
import jax.experimental.pallas.tpu as pltpu

_HG = 4
_NB = 3


@jax.jit
def pallas_concat_heads__mha_block_cached__gqa_block_cached__near_ridge_kernel(
    A_x: jax.Array,
    A_k_cache: jax.Array,
    A_v_cache: jax.Array,
    A_wq: jax.Array,
    A_wo: jax.Array,
    B_x: jax.Array,
    B_k_cache: jax.Array,
    B_v_cache: jax.Array,
    B_wq: jax.Array,
    B_wo: jax.Array,
):
    B, Sq, D = A_x.shape
    H, Sk, Dh = A_k_cache.shape[1:]
    assert B_k_cache.shape == A_k_cache.shape
    HG, NB = _HG, _NB
    NG = H // HG
    N = B * NG
    W = HG * Dh
    dt = A_x.dtype
    c = (Dh ** -0.5) * math.log2(math.e)

    def kernel(ax, ak, av, awq, awo, bx, bk, bv, bwq, bwo, o_hbm,
               xb, wqb, wob, kvb, acc, ob, sem, wsem, xsem, osem):
        br = ((ax, ak, av, awq, awo), (bx, bk, bv, bwq, bwo))

        def kv_copies(i, j):
            b, g, slot = i // NG, i % NG, i % NB
            return [
                pltpu.make_async_copy(br[j][1 + t].at[b, pl.ds(g * HG, HG)],
                                      kvb.at[slot, 2 * j + t], sem.at[slot, j])
                for t in range(2)
            ]

        def w_copies(g):
            off = pl.multiple_of(g * W, W)
            out = []
            for j in range(2):
                out.append(pltpu.make_async_copy(
                    br[j][3].at[:, pl.ds(off, W)], wqb.at[j, g], wsem.at[g]))
                out.append(pltpu.make_async_copy(
                    br[j][4].at[pl.ds(off, W), :], wob.at[j, g], wsem.at[g]))
            return out

        def x_copies(b):
            return [pltpu.make_async_copy(br[j][0].at[b], xb.at[j, b], xsem.at[b])
                    for j in range(2)]

        def o_copy(b):
            return pltpu.make_async_copy(ob.at[b], o_hbm.at[b], osem.at[b])

        def issue(i, j):
            if j == 0:
                @pl.when(i % NG == 0)
                def _():
                    for cp in x_copies(i // NG):
                        cp.start()

                @pl.when(i < NG)
                def _():
                    for cp in w_copies(i):
                        cp.start()
            for cp in kv_copies(i, j):
                cp.start()

        for i in range(NB - 1):
            for j in range(2):
                issue(jnp.int32(i), j)

        def batch_body(b, _):
            for cp in x_copies(b):
                cp.wait()
            acc[...] = jnp.zeros_like(acc)

            def group_body(g, _):
                i = b * NG + g
                n = i + NB - 1
                slot = i % NB
                for j in range(2):
                    @pl.when(n < N)
                    def _():
                        issue(n, j)

                    if j == 0:
                        @pl.when(b == 0)
                        def _():
                            for cp in w_copies(g):
                                cp.wait()
                    for cp in kv_copies(i, j):
                        cp.wait()

                    q = jnp.dot(xb[j, b], wqb[j, g], preferred_element_type=jnp.float32)
                    q = (q * c).astype(dt)
                    os_ = []
                    for h in range(HG):
                        s = jax.lax.dot_general(
                            q[:, h * Dh:(h + 1) * Dh], kvb[slot, 2 * j, h],
                            (((1,), (1,)), ((), ())),
                            preferred_element_type=jnp.float32)
                        m = jnp.max(s, axis=1, keepdims=True)
                        p = jnp.exp2(s - m)
                        l = jnp.sum(p, axis=1, keepdims=True)
                        o = jnp.dot(p.astype(dt), kvb[slot, 2 * j + 1, h],
                                    preferred_element_type=jnp.float32)
                        os_.append((o * (1.0 / l)).astype(dt))
                    acc[:, j * D:(j + 1) * D] += jnp.dot(
                        jnp.concatenate(os_, axis=1), wob[j, g],
                        preferred_element_type=jnp.float32)

            jax.lax.fori_loop(0, NG, group_body, None)
            ob[b] = acc[...].astype(dt)
            o_copy(b).start()

        jax.lax.fori_loop(0, B, batch_body, None)
        for b in range(B):
            o_copy(b).wait()

    any_spec = pl.BlockSpec(memory_space=pl.ANY)
    return pl.pallas_call(
        kernel,
        in_specs=[any_spec] * 10,
        out_specs=any_spec,
        out_shape=jax.ShapeDtypeStruct((B, Sq, 2 * D), dt),
        scratch_shapes=[
            pltpu.VMEM((2, B, Sq, D), dt),
            pltpu.VMEM((2, NG, D, W), dt),
            pltpu.VMEM((2, NG, W, D), dt),
            pltpu.VMEM((NB, 4, HG, Sk, Dh), dt),
            pltpu.VMEM((Sq, 2 * D), jnp.float32),
            pltpu.VMEM((B, Sq, 2 * D), dt),
            pltpu.SemaphoreType.DMA((NB, 2)),
            pltpu.SemaphoreType.DMA((NG,)),
            pltpu.SemaphoreType.DMA((B,)),
            pltpu.SemaphoreType.DMA((B,)),
        ],
        compiler_params=pltpu.CompilerParams(vmem_limit_bytes=100 * 2**20),
    )(A_x, A_k_cache, A_v_cache, A_wq, A_wo, B_x, B_k_cache, B_v_cache, B_wq, B_wo)
```
